```python
import jax
import jax.numpy as jnp

def _softmax(x, axis=-1):
    return jax.nn.softmax(x, axis=axis)
def _gelu(x):
    return jax.nn.gelu(x, approximate=True)
def _silu(x):
    return jax.nn.silu(x)
def _sigmoid(x):
    return jax.nn.sigmoid(x)
def _layernorm(x, axis=-1, eps=1e-5):
    m = jnp.mean(x, axis=axis, keepdims=True)
    v = jnp.var(x, axis=axis, keepdims=True)
    return (x - m) / jnp.sqrt(v + eps)
def _scatter_add(tgt, idx, src, axis=0):
    return tgt.at[idx].add(src)
def _segment_sum(src, seg, n):
    return jax.ops.segment_sum(src, seg, n)
class _Rng:
    def __init__(self, key):
        self._k = key
    def _next(self):
        self._k, sub = jax.random.split(self._k)
        return sub
    def normal(self, shape):
        return jax.random.normal(self._next(), shape, dtype=jnp.bfloat16)
    def randint(self, lo, hi, shape):
        return jax.random.randint(self._next(), shape, lo, hi, dtype=jnp.int32)
    def uniform(self, shape, lo=0.0, hi=1.0):
        return jax.random.uniform(self._next(), shape, jnp.bfloat16, lo, hi)
    def permutation(self, n):
        return jax.random.permutation(self._next(), n)


kernel_name = 'recurrent_scan__sliding_block_cached__moe_arch_mod__decode'

def setup_inputs():
    _rng = _Rng(jax.random.key(int.from_bytes(__import__("os").urandom(4), "little")))
    _w = (lambda a: (lambda t: t.astype(jnp.bfloat16) if jnp.issubdtype(t.dtype, jnp.floating) else t)(jnp.asarray(a)))
    def _A_setup():
        B, Sq, D = 1, 1, 512
        Hq, Hkv, Sk, Dh = 32, 32, 32768, 128
        assert Hq % Hkv == 0, (Hq, Hkv)
        return {
            "x": _w((lambda *s: _rng.normal(s) * 0.05)(B, Sq, D)),
            "k_cache": _w((lambda *s: _rng.normal(s) * 0.05)(B, Hkv, Sk, Dh)),
            "v_cache": _w((lambda *s: _rng.normal(s) * 0.05)(B, Hkv, Sk, Dh)),
            "wq": _w((lambda *s: _rng.normal(s) * 0.05)(D, Hq * Dh) * (D ** -0.5)),
            "wo": _w((lambda *s: _rng.normal(s) * 0.05)(Hq * Dh, D) * ((Hq * Dh) ** -0.5)),
        }
    _A_in = _A_setup()

    def _B_setup():
        B, S, D, F, C = 1, 1, 512, 1376, 1
        return {
            "x": _w((lambda *s: _rng.normal(s) * 0.05)(B, S, D)),
            "w_r": _w((lambda *s: _rng.normal(s) * 0.05)(D)),
            "w_gate": _w((lambda *s: _rng.normal(s) * 0.05)(D, F)),
            "w_up": _w((lambda *s: _rng.normal(s) * 0.05)(D, F)),
            "w_down": _w((lambda *s: _rng.normal(s) * 0.05)(F, D)),
        }
    _B_in = _B_setup()

    return {
        "A_x": _A_in["x"],
        "A_k_cache": _A_in["k_cache"],
        "A_v_cache": _A_in["v_cache"],
        "A_wq": _A_in["wq"],
        "A_wo": _A_in["wo"],
        "B_x": _B_in["x"],
        "B_w_r": _B_in["w_r"],
        "B_w_gate": _B_in["w_gate"],
        "B_w_up": _B_in["w_up"],
        "B_w_down": _B_in["w_down"],
    }

def reference(A_x, A_k_cache, A_v_cache, A_wq, A_wo, B_x, B_w_r, B_w_gate, B_w_up, B_w_down):
    def _A_ref(x, k_cache, v_cache, wq, wo):
        B, Sq, D = x.shape
        Hq, Dh = 32, 128
        Hkv, Sk = k_cache.shape[1], k_cache.shape[2]
        W = min(4096, max(256, Sk // 4))
        rep = Hq // Hkv
        q = (lambda x, *d: x.transpose(*d))((x @ wq).reshape(B, Sq, Hq, Dh), 0, 2, 1, 3)
        k = jnp.repeat(k_cache[:, :, Sk - W:, :], rep, axis=1)
        v = jnp.repeat(v_cache[:, :, Sk - W:, :], rep, axis=1)
        scores = jnp.einsum("bhqd,bhkd->bhqk", q, k) * (Dh ** -0.5)
        p = _softmax(scores, axis=-1)
        o = jnp.einsum("bhqk,bhkd->bhqd", p, v)
        return (lambda x, *d: x.transpose(*d))(o, 0, 2, 1, 3).reshape(B, Sq, Hq * Dh) @ wo

    def _B_ref(x, w_r, w_gate, w_up, w_down):
        B, S, D = x.shape
        C = 1
        r = x @ w_r
        idx = jnp.argsort(-r, axis=-1)[:, :C]
        idx_e = jnp.repeat(idx.reshape(B, C, 1), D, axis=2)
        x_sel = jnp.take_along_axis(x, idx_e, axis=1)
        g = _silu(x_sel @ w_gate)
        u = x_sel @ w_up
        y = (g * u) @ w_down
        r_sel = _sigmoid(jnp.take_along_axis(r, idx, axis=1))
        y = y * r_sel.reshape(B, C, 1)
        b_off = (jnp.arange(B) * S).reshape(B, 1)
        flat_idx = (idx + b_off).reshape(B * C)
        zero = (x * 0.0).reshape(B * S, D)
        upd = _scatter_add(zero, flat_idx, y.reshape(B * C, D), axis=0)
        return x + upd.reshape(B, S, D)

    x = A_x
    xn = _layernorm(x, axis=-1)
    s = _A_ref(xn, A_k_cache, A_v_cache, A_wq, A_wo)
    g = _silu(_B_ref(xn, B_w_r, B_w_gate, B_w_up, B_w_down))
    return x + s * g
```

```python
import jax
import jax.numpy as jnp
from jax import lax
import jax.experimental.pallas as pl
import jax.experimental.pallas.tpu as pltpu

_NT = (((1,), (1,)), ((), ()))
_NN = (((1,), (0,)), ((), ()))


@jax.jit
def pallas_recurrent_scan__sliding_block_cached__moe_arch_mod__decode_kernel(
    A_x, A_k_cache, A_v_cache, A_wq, A_wo, B_x, B_w_r, B_w_gate, B_w_up, B_w_down,
):
    B, Sq, D = A_x.shape
    assert B == 1 and Sq == 1
    H, Dh = 32, 128
    Hkv, Sk = A_k_cache.shape[1], A_k_cache.shape[2]
    assert Hkv == H
    W = min(4096, max(256, Sk // 4))
    F = B_w_gate.shape[1]
    f32, bf16 = jnp.float32, jnp.bfloat16
    M = 8
    scale = Dh ** -0.5

    GH = 4
    G = H // GH
    RB = 32
    BLK = W // GH
    WR = 32
    WO_CH = [(0, 2048), (2048, 3072), (3072, 3840), (3840, 4096)]
    S_X, S_WR, S_WQ, S_WG, S_WU, S_WD = 0, 1, 2, 3, 4, 5
    S_WO = 6
    S_KV = S_WO + len(WO_CH)
    NSEM = S_KV + G

    def kernel(x_hbm, k_hbm, v_hbm, wq_hbm, wo_hbm, wr_hbm, wg_hbm, wu_hbm, wd_hbm,
               o_ref,
               x_v, wr_v, wq_v, wo_v, wg_v, wu_v, wd_v, kv_v, q_s, o_s, sem):

        def wait_all(buf, s):
            pltpu.make_async_copy(buf, buf, sem.at[s]).wait()

        def issue_kv_block(j):
            g = j // GH
            r0 = (j % GH) * BLK
            h0 = g * GH

            def body(i, c):
                r = pl.multiple_of(r0 + i * RB, RB)
                for w, src in ((0, k_hbm), (1, v_hbm)):
                    pltpu.make_async_copy(
                        src.at[0, pl.ds(h0, GH), pl.ds(Sk - W + r, RB), :],
                        kv_v.at[g, w, :, pl.ds(r, RB), :],
                        sem.at[S_KV + g]).start(priority=w)
                return c
            lax.fori_loop(0, BLK // RB, body, 0, unroll=8)

        def issue_wo(c):
            lo, hi = WO_CH[c]
            half = (hi - lo) // 2

            def body(i, carry):
                for w in (0, 1):
                    r = pl.multiple_of(lo + w * half + i * WR, WR)
                    pltpu.make_async_copy(
                        wo_hbm.at[pl.ds(r, WR), :], wo_v.at[pl.ds(r, WR), :],
                        sem.at[S_WO + c]).start(priority=w)
                return carry
            lax.fori_loop(0, half // WR, body, 0, unroll=4)

        pltpu.make_async_copy(x_hbm, x_v, sem.at[S_X]).start()
        pltpu.make_async_copy(wr_hbm, wr_v, sem.at[S_WR]).start(priority=1)
        nf = F // WR
        QC = H * Dh // 2

        def wq_desc(i):
            r = pl.multiple_of((i // 2) * 8, 8)
            c = pl.multiple_of((i % 2) * QC, QC)
            pltpu.make_async_copy(
                wq_hbm.at[pl.ds(r, 8), pl.ds(c, QC)], wq_v.at[pl.ds(r, 8), pl.ds(c, QC)],
                sem.at[S_WQ]).start(priority=0)

        nq = (D // 8) * 2
        for t, (src, dst, s) in enumerate(((wg_hbm, wg_v, S_WG), (wu_hbm, wu_v, S_WU), (wd_hbm, wd_v, S_WD))):
            def body(i, c, t=t, src=src, dst=dst, s=s):
                r = pl.multiple_of(i * WR, WR)
                pltpu.make_async_copy(src.at[pl.ds(r, WR), :], dst.at[pl.ds(r, WR), :],
                                      sem.at[s]).start(priority=1)
                if t < 2:
                    wq_desc(t * nf + i)
                else:
                    @pl.when(2 * nf + i < nq)
                    def _():
                        wq_desc(2 * nf + i)
                return c
            lax.fori_loop(0, nf, body, 0)

        issue_kv_block(0)

        pltpu.make_async_copy(x_hbm, x_v, sem.at[S_X]).wait()
        x = x_v[0].astype(f32)
        mu = jnp.mean(x, axis=-1, keepdims=True)
        xc = x - mu
        var = jnp.mean(xc * xc, axis=-1, keepdims=True)
        xn = xc / jnp.sqrt(var + 1e-5)
        xn_b = jnp.broadcast_to(xn, (M, D)).astype(bf16)

        wait_all(wq_v, S_WQ)
        q = lax.dot_general(xn_b, wq_v[...], _NN, preferred_element_type=f32)
        for h in range(H):
            q_s[h] = q[:, h * Dh:(h + 1) * Dh]

        issue_kv_block(1)

        pltpu.make_async_copy(wr_hbm, wr_v, sem.at[S_WR]).wait()
        rr = jnp.zeros((1, Dh), f32)
        for j in range(D // Dh):
            rr = rr + xn[:, j * Dh:(j + 1) * Dh] * wr_v[j:j + 1, :].astype(f32)
        r = jnp.sum(rr, axis=-1, keepdims=True)
        wait_all(wg_v, S_WG)
        gt = lax.dot_general(xn_b, wg_v[...], _NT, preferred_element_type=f32)
        wait_all(wu_v, S_WU)
        up = lax.dot_general(xn_b, wu_v[...], _NT, preferred_element_type=f32)
        hid = (gt * jax.nn.sigmoid(gt) * up).astype(bf16)

        issue_kv_block(2)

        wait_all(wd_v, S_WD)
        y = lax.dot_general(hid, wd_v[...], _NN, preferred_element_type=f32)
        z = xn + y[0:1] * jax.nn.sigmoid(r)
        g_out = z * jax.nn.sigmoid(z)

        issue_kv_block(3)

        def head(h, carry):
            @pl.when(h < H - GH)
            def _():
                issue_kv_block(h + GH)

            @pl.when(h == H - GH)
            def _():
                issue_wo(0)

            @pl.when(h == H - GH + 1)
            def _():
                issue_wo(1)

            @pl.when(h == H - GH + 2)
            def _():
                for c in range(2, len(WO_CH)):
                    issue_wo(c)

            g = h // GH
            hh = h % GH

            @pl.when(hh == 0)
            def _():
                wait_all(kv_v.at[g], S_KV + g)

            qh = q_s[h].astype(bf16)
            s = lax.dot_general(qh, kv_v[g, 0, hh], _NT, preferred_element_type=f32) * scale
            m = jnp.max(s, axis=-1, keepdims=True)
            p = jnp.exp(s - m)
            l = jnp.sum(p, axis=-1, keepdims=True)
            o = lax.dot_general(p.astype(bf16), kv_v[g, 1, hh], _NN, preferred_element_type=f32)
            o_s[h] = o / l
            return carry

        lax.fori_loop(0, H, head, 0)

        acc = jnp.zeros((M, D), f32)
        for c, (lo, hi) in enumerate(WO_CH):
            oc = jnp.concatenate([o_s[h] for h in range(lo // Dh, hi // Dh)], axis=1).astype(bf16)
            wait_all(wo_v.at[pl.ds(lo, hi - lo), :], S_WO + c)
            acc = acc + lax.dot_general(oc, wo_v[lo:hi, :], _NN, preferred_element_type=f32)
        o_ref[0] = (x + acc[0:1] * g_out).astype(o_ref.dtype)

    any_spec = pl.BlockSpec(memory_space=pl.ANY)
    return pl.pallas_call(
        kernel,
        out_shape=jax.ShapeDtypeStruct((B, Sq, D), A_x.dtype),
        in_specs=[any_spec] * 9,
        out_specs=pl.BlockSpec(memory_space=pltpu.VMEM),
        scratch_shapes=[
            pltpu.VMEM((1, 1, D), bf16),
            pltpu.VMEM((D // Dh, Dh), bf16),
            pltpu.VMEM((D, H * Dh), bf16),
            pltpu.VMEM((H * Dh, D), bf16),
            pltpu.VMEM((F, D), bf16),
            pltpu.VMEM((F, D), bf16),
            pltpu.VMEM((F, D), bf16),
            pltpu.VMEM((G, 2, GH, W, Dh), bf16),
            pltpu.VMEM((H, M, Dh), f32),
            pltpu.VMEM((H, M, Dh), f32),
            pltpu.SemaphoreType.DMA((NSEM,)),
        ],
        compiler_params=pltpu.CompilerParams(
            vmem_limit_bytes=100 * 1024 * 1024,
            disable_semaphore_checks=True,
            disable_bounds_checks=True),
    )(A_x, A_k_cache, A_v_cache, A_wq, A_wo, B_w_r.reshape(D // Dh, Dh),
      B_w_gate.T, B_w_up.T, B_w_down)
```

```python
import jax
import jax.numpy as jnp
from jax import lax
import jax.experimental.pallas as pl
import jax.experimental.pallas.tpu as pltpu

_NT = (((1,), (1,)), ((), ()))
_NN = (((1,), (0,)), ((), ()))

GH = 4
RB = 40
LOOK = 5
FQ, FR = 2, 24
OQ, OR = 4, 8
QQ, QC = 4, 512
WO_CHUNKS = ((0, 320), (1, 160), (0, 256), (1, 160), (1, 64), (1, 32), (1, 32))
TRAIL_KIB = (5000, 600, 600, 600, 600, 450, 450)


def _spans(lo, hi, step):
    out = []
    while lo < hi:
        n = min(step, hi - lo)
        out.append((lo, n))
        lo += n
    return out


@jax.jit
def pallas_recurrent_scan__sliding_block_cached__moe_arch_mod__decode_kernel(
    A_x: jax.Array,
    A_k_cache: jax.Array,
    A_v_cache: jax.Array,
    A_wq: jax.Array,
    A_wo: jax.Array,
    B_x: jax.Array,
    B_w_r: jax.Array,
    B_w_gate: jax.Array,
    B_w_up: jax.Array,
    B_w_down: jax.Array,
):
    B, Sq, D = A_x.shape
    H, Dh = 32, 128
    Hkv, Sk = A_k_cache.shape[1], A_k_cache.shape[2]
    assert B == 1 and Sq == 1 and Hkv == H
    W = min(4096, max(256, Sk // 4))
    F = B_w_gate.shape[1]
    f32, bf16 = jnp.float32, jnp.bfloat16
    M = 8
    scale = Dh ** -0.5
    G = H // GH
    FS, OS, QS = F // FQ, H * Dh // OQ, D // QQ

    assert sum(n for _, n in WO_CHUNKS) == OS
    chunks = []
    nxt = [0, sum(n for t, n in WO_CHUNKS if t == 0)]
    for t, n in WO_CHUNKS:
        chunks.append((t, nxt[t], nxt[t] + n))
        nxt[t] += n
    NCH = len(chunks)
    S_X, S_WR, S_WQ, S_WG, S_WU, S_WD, S_WO = 0, 1, 2, 3, 4, 5, 6
    S_KV = S_WO + NCH
    NSEM = S_KV + G

    dsplit = (FS // 2 + 7) // 8 * 8
    streams = [
        [("g", r, n, S_WG) for r, n in _spans(0, FS, FR)]
        + [("d", r, n, S_WD) for r, n in _spans(0, dsplit, FR)],
        [("u", r, n, S_WU) for r, n in _spans(0, FS, FR)]
        + [("d", r, n, S_WD) for r, n in _spans(dsplit, FS, FR)],
    ]
    for c, (t, a0, a1) in enumerate(chunks):
        streams[t].extend([("o", r, n, S_WO + c) for r, n in _spans(a0, a1, OR)])
    trail = []
    for i in range(max(len(s) for s in streams)):
        for t in (0, 1):
            if i < len(streams[t]):
                trail.append(streams[t][i] + (t,))
    cuts = [0]
    for budget in TRAIL_KIB:
        i, used = cuts[-1], 0
        while i < len(trail) and used < budget:
            used += trail[i][2] * (OQ if trail[i][0] == "o" else FQ) * D * 2 // 1024
            i += 1
        cuts.append(i)
    cuts.append(len(trail))
    assert all(e[0] == "o" for e in trail[cuts[5]:])

    NB = W // RB
    REM = W - NB * RB
    PAIRS = -(-NB // (2 * GH))
    assert NB % 2 == 0 and RB % 8 == 0 and REM % 8 == 0 and LOOK >= GH

    def kernel(x_hbm, k_hbm, v_hbm, wq_hbm, wo_hbm, wr_hbm, wg_hbm, wu_hbm, wd_hbm,
               o_ref,
               x_v, wr_v, wq_v, wo_v, wg_v, wu_v, wd_v, kv_v, q_s, o_s, acc_s, sem):

        def wait_all(buf, s):
            pltpu.make_async_copy(buf, buf, sem.at[s]).wait()

        def issue_kv_block(j):
            g = j // GH
            jj = j % GH

            def copy_rows(r, n):
                for w, src in ((0, k_hbm), (1, v_hbm)):
                    pltpu.make_async_copy(
                        src.at[0, pl.ds(g * GH, GH), pl.ds(Sk - W + r, n), :],
                        kv_v.at[g, w, :, pl.ds(r, n), :],
                        sem.at[S_KV + g]).start(priority=w)

            def body(i, c):
                for u in range(2):
                    copy_rows(pl.multiple_of((2 * i + u) * RB, 8), RB)
                return c

            lo = jj * PAIRS
            lax.fori_loop(lo, jnp.minimum(lo + PAIRS, NB // 2), body, 0)
            if REM:
                @pl.when(jj == GH - 1)
                def _():
                    copy_rows(NB * RB, REM)

        arrs = {"g": (wg_hbm, wg_v), "u": (wu_hbm, wu_v), "d": (wd_hbm, wd_v), "o": (wo_hbm, wo_v)}

        def issue_trail(k):
            for a, r, n, s, p in trail[cuts[k]:cuts[k + 1]]:
                src, dst = arrs[a]
                pltpu.make_async_copy(src.at[:, pl.ds(r, n), :], dst.at[:, pl.ds(r, n), :],
                                      sem.at[s]).start(priority=p)

        cp_x = pltpu.make_async_copy(x_hbm, x_v, sem.at[S_X])
        cp_wr = pltpu.make_async_copy(wr_hbm, wr_v, sem.at[S_WR])
        cp_x.start(priority=0)
        cp_wr.start(priority=1)

        def wq_body(i, c):
            for col, n in _spans(0, H * Dh, QC):
                for p in (0, 1):
                    r = pl.multiple_of(p * (QS // 2) + i * 8, 8)
                    pltpu.make_async_copy(wq_hbm.at[:, pl.ds(r, 8), pl.ds(col, n)],
                                          wq_v.at[:, pl.ds(r, 8), pl.ds(col, n)],
                                          sem.at[S_WQ]).start(priority=p)
            return c

        lax.fori_loop(0, QS // 16, wq_body, 0)
        issue_kv_block(0)
        issue_kv_block(1)

        cp_x.wait()
        x = x_v[0].astype(f32)
        xc = x - jnp.mean(x, axis=-1, keepdims=True)
        var = jnp.mean(xc * xc, axis=-1, keepdims=True)
        xn = xc / jnp.sqrt(var + 1e-5)
        xn_b = jnp.broadcast_to(xn, (M, D)).astype(bf16)
        cp_wr.wait()
        rr = jnp.zeros((1, Dh), f32)
        for j in range(D // Dh):
            rr = rr + xn[:, j * Dh:(j + 1) * Dh] * wr_v[j:j + 1, :].astype(f32)
        r_gate = jax.nn.sigmoid(jnp.sum(rr, axis=-1, keepdims=True))

        wait_all(wq_v, S_WQ)
        q = lax.dot_general(xn_b, wq_v[...].reshape(D, H * Dh), _NN, preferred_element_type=f32)
        for h in range(H):
            q_s[h] = q[:, h * Dh:(h + 1) * Dh]

        for j in range(2, LOOK):
            issue_kv_block(j)

        def head(h, carry):
            @pl.when(h < H - LOOK)
            def _():
                issue_kv_block(h + LOOK)

            for k in range(GH):
                @pl.when(h == H - GH + k)
                def _():
                    issue_trail(k)

            g = h // GH
            hh = h % GH

            @pl.when(hh == 0)
            def _():
                wait_all(kv_v.at[g], S_KV + g)

            qh = q_s[h].astype(bf16)
            s = lax.dot_general(qh, kv_v[g, 0, hh], _NT, preferred_element_type=f32) * scale
            p = jnp.exp(s - jnp.max(s, axis=-1, keepdims=True))
            l = jnp.sum(p, axis=-1, keepdims=True)
            o = lax.dot_general(p.astype(bf16), kv_v[g, 1, hh], _NN, preferred_element_type=f32)
            o_s[h] = o / l
            return carry

        lax.fori_loop(0, H, head, 0)

        issue_trail(4)
        wait_all(wg_v, S_WG)
        gt = lax.dot_general(xn_b, wg_v[...].reshape(F, D), _NT, preferred_element_type=f32)
        gt = gt * jax.nn.sigmoid(gt)
        issue_trail(5)
        wait_all(wu_v, S_WU)
        up = lax.dot_general(xn_b, wu_v[...].reshape(F, D), _NT, preferred_element_type=f32)
        hid = (gt * up).astype(bf16)
        issue_trail(6)
        wait_all(wd_v, S_WD)
        y = lax.dot_general(hid, wd_v[...].reshape(F, D), _NN, preferred_element_type=f32)
        z = xn + y * r_gate
        gate = z * jax.nn.sigmoid(z)
        x_rep = jnp.broadcast_to(x, (M, D))
        issue_trail(7)

        o_all = jnp.concatenate([o_s[h] for h in range(H)], axis=1)
        lhs = [
            jnp.concatenate([o_all[:, i * OS + a0:i * OS + a1] for i in range(OQ)], axis=1).astype(bf16)
            for _, a0, a1 in chunks
        ]
        for c, (_, a0, a1) in enumerate(chunks):
            wait_all(wo_v.at[:, pl.ds(a0, a1 - a0), :], S_WO + c)
            part = lax.dot_general(lhs[c], wo_v[:, a0:a1, :].reshape(OQ * (a1 - a0), D), _NN,
                                   preferred_element_type=f32)
            if c == 0:
                acc_s[...] = part
            elif c < NCH - 1:
                acc_s[...] += part
            else:
                res = x_rep + (acc_s[...] + part) * gate
                o_ref[0] = res[0:1].astype(o_ref.dtype)

    any_spec = pl.BlockSpec(memory_space=pl.ANY)
    return pl.pallas_call(
        kernel,
        out_shape=jax.ShapeDtypeStruct((B, Sq, D), A_x.dtype),
        in_specs=[any_spec] * 9,
        out_specs=pl.BlockSpec(memory_space=pltpu.VMEM),
        scratch_shapes=[
            pltpu.VMEM((1, 1, D), bf16),
            pltpu.VMEM((D // Dh, Dh), bf16),
            pltpu.VMEM((QQ, QS, H * Dh), bf16),
            pltpu.VMEM((OQ, OS, D), bf16),
            pltpu.VMEM((FQ, FS, D), bf16),
            pltpu.VMEM((FQ, FS, D), bf16),
            pltpu.VMEM((FQ, FS, D), bf16),
            pltpu.VMEM((G, 2, GH, W, Dh), bf16),
            pltpu.VMEM((H, M, Dh), f32),
            pltpu.VMEM((H, M, Dh), f32),
            pltpu.VMEM((M, D), f32),
            pltpu.SemaphoreType.DMA((NSEM,)),
        ],
        compiler_params=pltpu.CompilerParams(
            vmem_limit_bytes=100 * 1024 * 1024,
            disable_semaphore_checks=True,
            disable_bounds_checks=True),
    )(A_x, A_k_cache, A_v_cache,
      A_wq.reshape(QQ, QS, H * Dh), A_wo.reshape(OQ, OS, D), B_w_r.reshape(D // Dh, Dh),
      B_w_gate.T.reshape(FQ, FS, D), B_w_up.T.reshape(FQ, FS, D), B_w_down.reshape(FQ, FS, D))
```

```python
import jax
import jax.numpy as jnp
from jax import lax
import jax.experimental.pallas as pl
import jax.experimental.pallas.tpu as pltpu

_NT = (((1,), (1,)), ((), ()))
_NN = (((1,), (0,)), ((), ()))

GH = 4
RB = 40
LOOK = 5
FQ, FR = 2, 24
OQ, OR = 4, 8
QQ, QC = 4, 512
QSM, QC0 = 2, 128
WO_CHUNKS = ((0, 256), (1, 224), (0, 256), (1, 160), (1, 64), (1, 32), (1, 24), (1, 8))
N_VPU = 2
TRAIL_KIB = (5000, 600, 600, 600, 600, 450, 450)


def _spans(lo, hi, step):
    out = []
    while lo < hi:
        n = min(step, hi - lo)
        out.append((lo, n))
        lo += n
    return out


@jax.jit
def pallas_recurrent_scan__sliding_block_cached__moe_arch_mod__decode_kernel(
    A_x: jax.Array,
    A_k_cache: jax.Array,
    A_v_cache: jax.Array,
    A_wq: jax.Array,
    A_wo: jax.Array,
    B_x: jax.Array,
    B_w_r: jax.Array,
    B_w_gate: jax.Array,
    B_w_up: jax.Array,
    B_w_down: jax.Array,
):
    B, Sq, D = A_x.shape
    H, Dh = 32, 128
    Hkv, Sk = A_k_cache.shape[1], A_k_cache.shape[2]
    assert B == 1 and Sq == 1 and Hkv == H
    W = min(4096, max(256, Sk // 4))
    F = B_w_gate.shape[1]
    f32, bf16 = jnp.float32, jnp.bfloat16
    M = 8
    scale = Dh ** -0.5
    G = H // GH
    FS, OS, QS = F // FQ, H * Dh // OQ, D // QQ

    assert sum(n for _, n in WO_CHUNKS) == OS
    chunks = []
    nxt = [0, sum(n for t, n in WO_CHUNKS if t == 0)]
    for t, n in WO_CHUNKS:
        chunks.append((t, nxt[t], nxt[t] + n))
        nxt[t] += n
    NCH = len(chunks)
    NMX = NCH - N_VPU
    v0, v1 = chunks[NMX][1], chunks[-1][2]
    NV = v1 - v0
    assert all(chunks[c][2] == chunks[c + 1][1] for c in range(NMX, NCH - 1))
    assert v0 // Dh == (v1 - 1) // Dh and OS % Dh == 0
    S_X, S_WR, S_WQ, S_WG, S_WU, S_WD, S_WO = 0, 1, 2, 3, 4, 5, 6
    S_KV = S_WO + NCH
    NSEM = S_KV + G

    dsplit = (FS // 2 + 7) // 8 * 8
    streams = [
        [("g", r, n, S_WG) for r, n in _spans(0, FS, FR)]
        + [("d", r, n, S_WD) for r, n in _spans(0, dsplit, FR)],
        [("u", r, n, S_WU) for r, n in _spans(0, FS, FR)]
        + [("d", r, n, S_WD) for r, n in _spans(dsplit, FS, FR)],
    ]
    for c, (t, a0, a1) in enumerate(chunks):
        streams[t].extend([("o", r, n, S_WO + c) for r, n in _spans(a0, a1, OR)])
    trail = []
    for i in range(max(len(s) for s in streams)):
        for t in (0, 1):
            if i < len(streams[t]):
                trail.append(streams[t][i] + (t,))
    cuts = [0]
    for budget in TRAIL_KIB:
        i, used = cuts[-1], 0
        while i < len(trail) and used < budget:
            used += trail[i][2] * (OQ if trail[i][0] == "o" else FQ) * D * 2 // 1024
            i += 1
        cuts.append(i)
    cuts.append(len(trail))
    assert all(e[0] == "o" for e in trail[cuts[5]:])

    NB = W // RB
    REM = W - NB * RB
    PAIRS = -(-NB // (2 * GH))
    assert NB % 2 == 0 and RB % 8 == 0 and REM % 8 == 0 and LOOK >= GH

    def kernel(x_hbm, k_hbm, v_hbm, wq_hbm, wo_hbm, wr_hbm, wg_hbm, wu_hbm, wd_hbm,
               o_ref,
               x_v, wr_v, wq_v, wo_v, wg_v, wu_v, wd_v, kv_v, q_s, o_s, acc_s, oc_s, sem):

        def wait_all(buf, s):
            pltpu.make_async_copy(buf, buf, sem.at[s]).wait()

        def issue_kv_block(j):
            g = j // GH
            jj = j % GH

            def copy_rows(r, n):
                for w, src in ((0, k_hbm), (1, v_hbm)):
                    pltpu.make_async_copy(
                        src.at[0, pl.ds(g * GH, GH), pl.ds(Sk - W + r, n), :],
                        kv_v.at[g, w, :, pl.ds(r, n), :],
                        sem.at[S_KV + g]).start(priority=w)

            def body(i, c):
                for u in range(2):
                    copy_rows(pl.multiple_of((2 * i + u) * RB, 8), RB)
                return c

            lo = jj * PAIRS
            lax.fori_loop(lo, jnp.minimum(lo + PAIRS, NB // 2), body, 0)
            if REM:
                @pl.when(jj == GH - 1)
                def _():
                    copy_rows(NB * RB, REM)

        arrs = {"g": (wg_hbm, wg_v), "u": (wu_hbm, wu_v), "d": (wd_hbm, wd_v), "o": (wo_hbm, wo_v)}

        def issue_trail(k):
            for a, r, n, s, p in trail[cuts[k]:cuts[k + 1]]:
                src, dst = arrs[a]
                pltpu.make_async_copy(src.at[:, pl.ds(r, n), :], dst.at[:, pl.ds(r, n), :],
                                      sem.at[s]).start(priority=p)

        cp_x = pltpu.make_async_copy(x_hbm, x_v, sem.at[S_X])
        cp_wr = pltpu.make_async_copy(wr_hbm, wr_v, sem.at[S_WR])
        cp_x.start(priority=0)
        cp_wr.start(priority=1)

        def copy_wq(tile, col, n):
            for p in (0, 1):
                r = pl.multiple_of(p * (QS // 2) + tile * 8, 8)
                pltpu.make_async_copy(wq_hbm.at[:, pl.ds(r, 8), pl.ds(col, n)],
                                      wq_v.at[:, pl.ds(r, 8), pl.ds(col, n)],
                                      sem.at[S_WQ]).start(priority=p)

        def wq_small(j, c):
            per_tile = H * Dh // QC0
            copy_wq(j // per_tile, pl.multiple_of((j % per_tile) * QC0, QC0), QC0)
            return c

        def wq_body(i, c):
            for col, n in _spans(0, H * Dh, QC):
                copy_wq(i, col, n)
            return c

        lax.fori_loop(0, QSM * (H * Dh // QC0), wq_small, 0)
        lax.fori_loop(QSM, QS // 16, wq_body, 0)
        issue_kv_block(0)
        issue_kv_block(1)

        cp_x.wait()
        x = x_v[0].astype(f32)
        xc = x - jnp.mean(x, axis=-1, keepdims=True)
        var = jnp.mean(xc * xc, axis=-1, keepdims=True)
        xn = xc / jnp.sqrt(var + 1e-5)
        xn_b = jnp.broadcast_to(xn, (M, D)).astype(bf16)
        cp_wr.wait()
        rr = jnp.zeros((1, Dh), f32)
        for j in range(D // Dh):
            rr = rr + xn[:, j * Dh:(j + 1) * Dh] * wr_v[j:j + 1, :].astype(f32)
        r_gate = jax.nn.sigmoid(jnp.sum(rr, axis=-1, keepdims=True))

        wait_all(wq_v, S_WQ)
        q = lax.dot_general(xn_b, wq_v[...].reshape(D, H * Dh), _NN, preferred_element_type=f32)
        for h in range(H):
            q_s[h] = q[:, h * Dh:(h + 1) * Dh]

        for j in range(2, LOOK):
            issue_kv_block(j)

        def head(h, carry):
            @pl.when(h < H - LOOK)
            def _():
                issue_kv_block(h + LOOK)

            for k in range(GH):
                @pl.when(h == H - GH + k)
                def _():
                    issue_trail(k)

            g = h // GH
            hh = h % GH

            @pl.when(hh == 0)
            def _():
                wait_all(kv_v.at[g], S_KV + g)

            qh = q_s[h].astype(bf16)
            s = lax.dot_general(qh, kv_v[g, 0, hh], _NT, preferred_element_type=f32) * scale
            p = jnp.exp(s - jnp.max(s, axis=-1, keepdims=True))
            l = jnp.sum(p, axis=-1, keepdims=True)
            o = lax.dot_general(p.astype(bf16), kv_v[g, 1, hh], _NN, preferred_element_type=f32)
            o_s[h] = o / l
            return carry

        lax.fori_loop(0, H, head, 0)

        issue_trail(4)
        wait_all(wg_v, S_WG)
        gt = lax.dot_general(xn_b, wg_v[...].reshape(F, D), _NT, preferred_element_type=f32)
        gt = gt * jax.nn.sigmoid(gt)
        issue_trail(5)
        wait_all(wu_v, S_WU)
        up = lax.dot_general(xn_b, wu_v[...].reshape(F, D), _NT, preferred_element_type=f32)
        hid = (gt * up).astype(bf16)
        issue_trail(6)
        wait_all(wd_v, S_WD)
        y = lax.dot_general(hid, wd_v[...].reshape(F, D), _NN, preferred_element_type=f32)
        z = xn + y * r_gate
        gate = z * jax.nn.sigmoid(z)
        x_rep = jnp.broadcast_to(x, (M, D))
        issue_trail(7)

        o_all = jnp.concatenate([o_s[h] for h in range(H)], axis=1)
        lhs = [
            jnp.concatenate([o_all[:, i * OS + a0:i * OS + a1] for i in range(OQ)], axis=1).astype(bf16)
            for _, a0, a1 in chunks[:NMX]
        ]
        pick = (lax.broadcasted_iota(jnp.int32, (NV, Dh), 1)
                == lax.broadcasted_iota(jnp.int32, (NV, Dh), 0) + v0 % Dh)
        diag = jnp.concatenate([
            jnp.where(pick, jnp.broadcast_to(o_s[(i * OS + v0) // Dh][0:1], (NV, Dh)), 0.0)
            for i in range(OQ)], axis=0).astype(bf16)
        oc_s[...] = lax.dot_general(diag, jnp.ones((Dh, Dh), bf16), _NN, preferred_element_type=f32)

        for c, (_, a0, a1) in enumerate(chunks[:NMX]):
            wait_all(wo_v.at[:, pl.ds(a0, a1 - a0), :], S_WO + c)
            part = lax.dot_general(lhs[c], wo_v[:, a0:a1, :].reshape(OQ * (a1 - a0), D), _NN,
                                   preferred_element_type=f32)
            if c == 0:
                acc_s[...] = part
            elif c < NMX - 1:
                acc_s[...] += part
            else:
                res = x_rep + (acc_s[...] + part) * gate

        terms = []
        for c in range(NMX, NCH):
            _, a0, a1 = chunks[c]
            wait_all(wo_v.at[:, pl.ds(a0, a1 - a0), :], S_WO + c)
            for i in range(OQ):
                for r in range(a0, a1, 8):
                    oc = oc_s[pl.ds(i * NV + r - v0, 8), :]
                    terms.insert(0, wo_v[i, r:r + 8, :].astype(f32)
                                 * jnp.concatenate([oc] * (D // Dh), axis=1))
            while len(terms) > 1:
                terms = [terms[k] + terms[k + 1] if k + 1 < len(terms) else terms[k]
                         for k in range(0, len(terms), 2)]
        res = res[0:1] + jnp.sum(terms[0], axis=0, keepdims=True) * gate[0:1]
        o_ref[0] = res.astype(o_ref.dtype)

    params = dict(vmem_limit_bytes=100 * 1024 * 1024, disable_bounds_checks=True)
    try:
        compiler_params = pltpu.CompilerParams(disable_semaphore_checks=True, **params)
    except TypeError:
        compiler_params = pltpu.CompilerParams(**params)

    any_spec = pl.BlockSpec(memory_space=pl.ANY)
    return pl.pallas_call(
        kernel,
        out_shape=jax.ShapeDtypeStruct((B, Sq, D), A_x.dtype),
        in_specs=[any_spec] * 9,
        out_specs=pl.BlockSpec(memory_space=pltpu.VMEM),
        scratch_shapes=[
            pltpu.VMEM((1, 1, D), bf16),
            pltpu.VMEM((D // Dh, Dh), bf16),
            pltpu.VMEM((QQ, QS, H * Dh), bf16),
            pltpu.VMEM((OQ, OS, D), bf16),
            pltpu.VMEM((FQ, FS, D), bf16),
            pltpu.VMEM((FQ, FS, D), bf16),
            pltpu.VMEM((FQ, FS, D), bf16),
            pltpu.VMEM((G, 2, GH, W, Dh), bf16),
            pltpu.VMEM((H, M, Dh), f32),
            pltpu.VMEM((H, M, Dh), f32),
            pltpu.VMEM((M, D), f32),
            pltpu.VMEM((OQ * NV, Dh), f32),
            pltpu.SemaphoreType.DMA((NSEM,)),
        ],
        compiler_params=compiler_params,
    )(A_x, A_k_cache, A_v_cache,
      A_wq.reshape(QQ, QS, H * Dh), A_wo.reshape(OQ, OS, D), B_w_r.reshape(D // Dh, Dh),
      B_w_gate.T.reshape(FQ, FS, D), B_w_up.T.reshape(FQ, FS, D), B_w_down.reshape(FQ, FS, D))
```

```python
import jax
import jax.numpy as jnp
from jax import lax
import jax.experimental.pallas as pl
import jax.experimental.pallas.tpu as pltpu

_NT = (((1,), (1,)), ((), ()))
_NN = (((1,), (0,)), ((), ()))

GH = 4
RB = 40
LOOK = 6
QQ = 4
QSM, QC0 = 2, 128
GR = 32
GU_FIRST = 64
GU_HEAD = 16
DQ, DR = 2, 24
OQ, OR = 4, 8
WO_CHUNKS = ((0, 256), (1, 224), (0, 256), (1, 160), (1, 64), (1, 32), (1, 24), (1, 8))
N_VPU = 2
TRAIL_KIB = (3900, 650, 650, 650)


def _spans(lo, hi, step):
    out = []
    while lo < hi:
        n = min(step, hi - lo)
        out.append((lo, n))
        lo += n
    return out


@jax.jit
def pallas_recurrent_scan__sliding_block_cached__moe_arch_mod__decode_kernel(
    A_x: jax.Array,
    A_k_cache: jax.Array,
    A_v_cache: jax.Array,
    A_wq: jax.Array,
    A_wo: jax.Array,
    B_x: jax.Array,
    B_w_r: jax.Array,
    B_w_gate: jax.Array,
    B_w_up: jax.Array,
    B_w_down: jax.Array,
):
    B, Sq, D = A_x.shape
    H, Dh = 32, 128
    Hkv, Sk = A_k_cache.shape[1], A_k_cache.shape[2]
    assert B == 1 and Sq == 1 and Hkv == H
    W = min(4096, max(256, Sk // 4))
    F = B_w_gate.shape[1]
    f32, bf16 = jnp.float32, jnp.bfloat16
    M = 8
    scale = Dh ** -0.5
    G = H // GH
    DS, OS, QS = F // DQ, H * Dh // OQ, D // QQ

    assert sum(n for _, n in WO_CHUNKS) == OS
    chunks = []
    nxt = [0, sum(n for t, n in WO_CHUNKS if t == 0)]
    for t, n in WO_CHUNKS:
        chunks.append((t, nxt[t], nxt[t] + n))
        nxt[t] += n
    NCH = len(chunks)
    NMX = NCH - N_VPU
    v0, v1 = chunks[NMX][1], chunks[-1][2]
    NV = v1 - v0
    assert all(chunks[c][2] == chunks[c + 1][1] for c in range(NMX, NCH - 1))
    assert v0 // Dh == (v1 - 1) // Dh and OS % Dh == 0
    S_X, S_WR, S_WQ, S_WG, S_WU, S_WD, S_WO = 0, 1, 2, 3, 4, 5, 6
    S_KV = S_WO + NCH
    NSEM = S_KV + G

    dsplit = (DS // 2 + 7) // 8 * 8
    streams = [[("d", r, n, S_WD) for r, n in _spans(0, dsplit, DR)],
               [("d", r, n, S_WD) for r, n in _spans(dsplit, DS, DR)]]
    for c, (t, a0, a1) in enumerate(chunks):
        streams[t].extend([("o", r, n, S_WO + c) for r, n in _spans(a0, a1, OR)])
    trail = []
    for i in range(max(len(s) for s in streams)):
        for t in (0, 1):
            if i < len(streams[t]):
                trail.append(streams[t][i] + (t,))
    cuts = [0]
    for budget in TRAIL_KIB:
        i, used = cuts[-1], 0
        while i < len(trail) and used < budget:
            used += trail[i][2] * (OQ if trail[i][0] == "o" else DQ) * D * 2 // 1024
            i += 1
        cuts.append(i)
    cuts.append(len(trail))

    NB = W // RB
    REM = W - NB * RB
    STEPS = NB // 2
    PER_BLOCK = -(-STEPS // GH)
    NGU = F // GR
    QH = H * Dh // 2
    QT = QS // 16 - QSM
    assert NB % 2 == 0 and RB % 8 == 0 and REM % 8 == 0 and F % GR == 0 and len(TRAIL_KIB) == GH
    assert LOOK >= GH and 2 * QT * QQ <= STEPS
    assert STEPS <= GU_FIRST and GU_FIRST + NGU <= (GU_HEAD // GH) * STEPS

    def kernel(x_hbm, k_hbm, v_hbm, wq_hbm, wo_hbm, wr_hbm, wg_hbm, wu_hbm, wd_hbm,
               o_ref,
               x_v, wr_v, wq_v, wo_v, wg_v, wu_v, wd_v, kv_v,
               q_s, o_s, acc_s, oc_s, xn_s, hid_s, sem):

        def wait_all(buf, s):
            pltpu.make_async_copy(buf, buf, sem.at[s]).wait()

        def copy_kv(g, r, n):
            for p, src in ((0, k_hbm), (1, v_hbm)):
                pltpu.make_async_copy(
                    src.at[0, pl.ds(g * GH, GH), pl.ds(Sk - W + r, n), :],
                    kv_v.at[g, p, :, pl.ds(r, n), :],
                    sem.at[S_KV + g]).start(priority=p)

        def copy_wq(slabs, tile, col, n):
            for p in (0, 1):
                r = pl.multiple_of(p * (QS // 2) + tile * 8, 8)
                pltpu.make_async_copy(wq_hbm.at[slabs, pl.ds(r, 8), pl.ds(col, n)],
                                      wq_v.at[slabs, pl.ds(r, 8), pl.ds(col, n)],
                                      sem.at[S_WQ]).start(priority=p)

        def kv_steps(g, lo, hi, mix_in):
            def body(i, c):
                copy_kv(g, pl.multiple_of(2 * i * RB, 8), RB)
                mix_in(i)
                copy_kv(g, pl.multiple_of((2 * i + 1) * RB, 8), RB)
                return c

            lax.fori_loop(lo, hi, body, 0)

        def issue_kv_block(j):
            g = j // GH
            jj = j % GH

            def mix_gate_up(i):
                e = g * STEPS + i - GU_FIRST

                @pl.when(jnp.logical_and(e >= 0, e < NGU))
                def _():
                    rows = pl.ds(pl.multiple_of(e * GR, GR), GR)
                    pltpu.make_async_copy(wg_hbm.at[rows, :], wg_v.at[rows, :],
                                          sem.at[S_WG]).start(priority=0)
                    pltpu.make_async_copy(wu_hbm.at[rows, :], wu_v.at[rows, :],
                                          sem.at[S_WU]).start(priority=1)

            lo = jj * PER_BLOCK
            kv_steps(g, lo, jnp.minimum(lo + PER_BLOCK, STEPS), mix_gate_up)
            if REM:
                @pl.when(jj == GH - 1)
                def _():
                    copy_kv(g, NB * RB, REM)

        def issue_trail(k):
            for a, r, n, s, p in trail[cuts[k]:cuts[k + 1]]:
                src, dst = (wo_hbm, wo_v) if a == "o" else (wd_hbm, wd_v)
                pltpu.make_async_copy(src.at[:, pl.ds(r, n), :], dst.at[:, pl.ds(r, n), :],
                                      sem.at[s]).start(priority=p)

        cp_x = pltpu.make_async_copy(x_hbm, x_v, sem.at[S_X])
        cp_wr = pltpu.make_async_copy(wr_hbm, wr_v, sem.at[S_WR])
        cp_x.start(priority=0)
        cp_wr.start(priority=1)

        def wq_small(j, c):
            per_tile = H * Dh // QC0
            copy_wq(slice(None), j // per_tile, pl.multiple_of((j % per_tile) * QC0, QC0), QC0)
            return c

        lax.fori_loop(0, QSM * (H * Dh // QC0), wq_small, 0)

        def mix_wq(i):
            @pl.when(i < 2 * QT * QQ)
            def _():
                k = i % (2 * QT)
                copy_wq(i // (2 * QT), QSM + k // 2, pl.multiple_of((k % 2) * QH, QH), QH)

        kv_steps(0, 0, STEPS, mix_wq)
        if REM:
            copy_kv(0, NB * RB, REM)

        cp_x.wait()
        x = x_v[0].astype(f32)
        xc = x - jnp.mean(x, axis=-1, keepdims=True)
        var = jnp.mean(xc * xc, axis=-1, keepdims=True)
        xn = xc / jnp.sqrt(var + 1e-5)
        xn_s[...] = jnp.broadcast_to(xn, (M, D))
        cp_wr.wait()
        rr = jnp.zeros((1, Dh), f32)
        for j in range(D // Dh):
            rr = rr + xn[:, j * Dh:(j + 1) * Dh] * wr_v[j:j + 1, :].astype(f32)
        r_gate = jax.nn.sigmoid(jnp.sum(rr, axis=-1, keepdims=True))

        for j in range(GH, LOOK):
            issue_kv_block(j)

        wait_all(wq_v, S_WQ)
        q = lax.dot_general(xn_s[...].astype(bf16), wq_v[...].reshape(D, H * Dh), _NN,
                            preferred_element_type=f32)
        for h in range(H):
            q_s[h] = q[:, h * Dh:(h + 1) * Dh]

        def head(h, carry):
            @pl.when(h < H - LOOK)
            def _():
                issue_kv_block(h + LOOK)

            for k in range(GH):
                @pl.when(h == H - GH + k)
                def _():
                    issue_trail(k)

            @pl.when(h == GU_HEAD)
            def _():
                xb = xn_s[...].astype(bf16)
                wait_all(wg_v, S_WG)
                gt = lax.dot_general(xb, wg_v[...], _NT, preferred_element_type=f32)
                gt = gt * jax.nn.sigmoid(gt)
                wait_all(wu_v, S_WU)
                up = lax.dot_general(xb, wu_v[...], _NT, preferred_element_type=f32)
                hid_s[...] = gt * up

            g = h // GH
            hh = h % GH

            @pl.when(hh == 0)
            def _():
                wait_all(kv_v.at[g], S_KV + g)

            qh = q_s[h].astype(bf16)
            s = lax.dot_general(qh, kv_v[g, 0, hh], _NT, preferred_element_type=f32) * scale
            p = jnp.exp(s - jnp.max(s, axis=-1, keepdims=True))
            l = jnp.sum(p, axis=-1, keepdims=True)
            o = lax.dot_general(p.astype(bf16), kv_v[g, 1, hh], _NN, preferred_element_type=f32)
            o_s[h] = o / l
            return carry

        lax.fori_loop(0, H, head, 0)

        issue_trail(GH)
        wait_all(wd_v, S_WD)
        y = lax.dot_general(hid_s[...].astype(bf16), wd_v[...].reshape(F, D), _NN,
                            preferred_element_type=f32)
        z = xn + y * r_gate
        gate = z * jax.nn.sigmoid(z)
        x_rep = jnp.broadcast_to(x, (M, D))

        o_all = jnp.concatenate([o_s[h] for h in range(H)], axis=1)
        lhs = [
            jnp.concatenate([o_all[:, i * OS + a0:i * OS + a1] for i in range(OQ)], axis=1).astype(bf16)
            for _, a0, a1 in chunks[:NMX]
        ]
        pick = (lax.broadcasted_iota(jnp.int32, (NV, Dh), 1)
                == lax.broadcasted_iota(jnp.int32, (NV, Dh), 0) + v0 % Dh)
        diag = jnp.concatenate([
            jnp.where(pick, jnp.broadcast_to(o_s[(i * OS + v0) // Dh][0:1], (NV, Dh)), 0.0)
            for i in range(OQ)], axis=0).astype(bf16)
        oc_s[...] = lax.dot_general(diag, jnp.ones((Dh, Dh), bf16), _NN, preferred_element_type=f32)

        for c, (_, a0, a1) in enumerate(chunks[:NMX]):
            wait_all(wo_v.at[:, pl.ds(a0, a1 - a0), :], S_WO + c)
            part = lax.dot_general(lhs[c], wo_v[:, a0:a1, :].reshape(OQ * (a1 - a0), D), _NN,
                                   preferred_element_type=f32)
            if c == 0:
                acc_s[...] = part
            elif c < NMX - 1:
                acc_s[...] += part
            else:
                res = x_rep + (acc_s[...] + part) * gate

        terms = []
        for c in range(NMX, NCH):
            _, a0, a1 = chunks[c]
            wait_all(wo_v.at[:, pl.ds(a0, a1 - a0), :], S_WO + c)
            for i in range(OQ):
                for r in range(a0, a1, 8):
                    oc = oc_s[pl.ds(i * NV + r - v0, 8), :]
                    terms.insert(0, wo_v[i, r:r + 8, :].astype(f32)
                                 * jnp.concatenate([oc] * (D // Dh), axis=1))
            while len(terms) > 1:
                terms = [terms[k] + terms[k + 1] if k + 1 < len(terms) else terms[k]
                         for k in range(0, len(terms), 2)]
        res = res[0:1] + jnp.sum(terms[0], axis=0, keepdims=True) * gate[0:1]
        o_ref[0] = res.astype(o_ref.dtype)

    params = dict(vmem_limit_bytes=100 * 1024 * 1024, disable_bounds_checks=True)
    try:
        compiler_params = pltpu.CompilerParams(disable_semaphore_checks=True, **params)
    except TypeError:
        compiler_params = pltpu.CompilerParams(**params)

    any_spec = pl.BlockSpec(memory_space=pl.ANY)
    return pl.pallas_call(
        kernel,
        out_shape=jax.ShapeDtypeStruct((B, Sq, D), A_x.dtype),
        in_specs=[any_spec] * 9,
        out_specs=pl.BlockSpec(memory_space=pltpu.VMEM),
        scratch_shapes=[
            pltpu.VMEM((1, 1, D), bf16),
            pltpu.VMEM((D // Dh, Dh), bf16),
            pltpu.VMEM((QQ, QS, H * Dh), bf16),
            pltpu.VMEM((OQ, OS, D), bf16),
            pltpu.VMEM((F, D), bf16),
            pltpu.VMEM((F, D), bf16),
            pltpu.VMEM((DQ, DS, D), bf16),
            pltpu.VMEM((G, 2, GH, W, Dh), bf16),
            pltpu.VMEM((H, M, Dh), f32),
            pltpu.VMEM((H, M, Dh), f32),
            pltpu.VMEM((M, D), f32),
            pltpu.VMEM((OQ * NV, Dh), f32),
            pltpu.VMEM((M, D), f32),
            pltpu.VMEM((M, F), f32),
            pltpu.SemaphoreType.DMA((NSEM,)),
        ],
        compiler_params=compiler_params,
    )(A_x, A_k_cache, A_v_cache,
      A_wq.reshape(QQ, QS, H * Dh), A_wo.reshape(OQ, OS, D), B_w_r.reshape(D // Dh, Dh),
      B_w_gate.T, B_w_up.T, B_w_down.reshape(DQ, DS, D))
```

```python
import jax
import jax.numpy as jnp
import numpy as np
from jax import lax
import jax.experimental.pallas as pl
import jax.experimental.pallas.tpu as pltpu

_NT = (((1,), (1,)), ((), ()))
_NN = (((1,), (0,)), ((), ()))

GH = 4
RB = 40
LOOK = 6
QQ = 4
QSM, QC0 = 2, 128
GR = 32
GU_FIRST = 64
GU_HEAD = 16
DQ, DR = 2, 24
OQ, OR = 4, 8
WO_CHUNKS = ((0, 256), (1, 224), (0, 256), (1, 160), (1, 64), (1, 32), (1, 24), (1, 8))
N_VPU = 2
TRAIL_KIB = (3900, 650, 650, 650)


def _rnd(a):
    return a.astype(jnp.bfloat16).astype(jnp.float32)


def _bf16_const(v):
    return float(np.asarray(v, dtype=jnp.bfloat16))


def _spans(lo, hi, step):
    out = []
    while lo < hi:
        n = min(step, hi - lo)
        out.append((lo, n))
        lo += n
    return out


@jax.jit
def pallas_recurrent_scan__sliding_block_cached__moe_arch_mod__decode_kernel(
    A_x: jax.Array,
    A_k_cache: jax.Array,
    A_v_cache: jax.Array,
    A_wq: jax.Array,
    A_wo: jax.Array,
    B_x: jax.Array,
    B_w_r: jax.Array,
    B_w_gate: jax.Array,
    B_w_up: jax.Array,
    B_w_down: jax.Array,
):
    B, Sq, D = A_x.shape
    H, Dh = 32, 128
    Hkv, Sk = A_k_cache.shape[1], A_k_cache.shape[2]
    assert B == 1 and Sq == 1 and Hkv == H
    W = min(4096, max(256, Sk // 4))
    F = B_w_gate.shape[1]
    f32, bf16 = jnp.float32, jnp.bfloat16
    M = 8
    scale = _bf16_const(Dh ** -0.5)
    eps = _bf16_const(1e-5)
    G = H // GH
    DS, OS, QS = F // DQ, H * Dh // OQ, D // QQ

    assert sum(n for _, n in WO_CHUNKS) == OS
    chunks = []
    nxt = [0, sum(n for t, n in WO_CHUNKS if t == 0)]
    for t, n in WO_CHUNKS:
        chunks.append((t, nxt[t], nxt[t] + n))
        nxt[t] += n
    NCH = len(chunks)
    NMX = NCH - N_VPU
    v0, v1 = chunks[NMX][1], chunks[-1][2]
    NV = v1 - v0
    assert all(chunks[c][2] == chunks[c + 1][1] for c in range(NMX, NCH - 1))
    assert v0 // Dh == (v1 - 1) // Dh and OS % Dh == 0
    S_X, S_WR, S_WQ, S_WG, S_WU, S_WD, S_WO = 0, 1, 2, 3, 4, 5, 6
    S_KV = S_WO + NCH
    NSEM = S_KV + G

    dsplit = (DS // 2 + 7) // 8 * 8
    streams = [[("d", r, n, S_WD) for r, n in _spans(0, dsplit, DR)],
               [("d", r, n, S_WD) for r, n in _spans(dsplit, DS, DR)]]
    for c, (t, a0, a1) in enumerate(chunks):
        streams[t].extend([("o", r, n, S_WO + c) for r, n in _spans(a0, a1, OR)])
    trail = []
    for i in range(max(len(s) for s in streams)):
        for t in (0, 1):
            if i < len(streams[t]):
                trail.append(streams[t][i] + (t,))
    cuts = [0]
    for budget in TRAIL_KIB:
        i, used = cuts[-1], 0
        while i < len(trail) and used < budget:
            used += trail[i][2] * (OQ if trail[i][0] == "o" else DQ) * D * 2 // 1024
            i += 1
        cuts.append(i)
    cuts.append(len(trail))

    NB = W // RB
    REM = W - NB * RB
    STEPS = NB // 2
    PER_BLOCK = -(-STEPS // GH)
    NGU = F // GR
    QH = H * Dh // 2
    QT = QS // 16 - QSM
    assert NB % 2 == 0 and RB % 8 == 0 and REM % 8 == 0 and F % GR == 0 and len(TRAIL_KIB) == GH
    assert LOOK >= GH and 2 * QT * QQ <= STEPS
    assert STEPS <= GU_FIRST and GU_FIRST + NGU <= (GU_HEAD // GH) * STEPS

    def kernel(x_hbm, k_hbm, v_hbm, wq_hbm, wo_hbm, wr_hbm, wg_hbm, wu_hbm, wd_hbm,
               o_ref,
               x_v, wr_v, wq_v, wo_v, wg_v, wu_v, wd_v, kv_v,
               q_s, o_s, acc_s, oc_s, xn_s, hid_s, sem):

        def wait_all(buf, s):
            pltpu.make_async_copy(buf, buf, sem.at[s]).wait()

        def copy_kv(g, r, n):
            for p, src in ((0, k_hbm), (1, v_hbm)):
                pltpu.make_async_copy(
                    src.at[0, pl.ds(g * GH, GH), pl.ds(Sk - W + r, n), :],
                    kv_v.at[g, p, :, pl.ds(r, n), :],
                    sem.at[S_KV + g]).start(priority=p)

        def copy_wq(slabs, tile, col, n):
            for p in (0, 1):
                r = pl.multiple_of(p * (QS // 2) + tile * 8, 8)
                pltpu.make_async_copy(wq_hbm.at[slabs, pl.ds(r, 8), pl.ds(col, n)],
                                      wq_v.at[slabs, pl.ds(r, 8), pl.ds(col, n)],
                                      sem.at[S_WQ]).start(priority=p)

        def kv_steps(g, lo, hi, mix_in):
            def body(i, c):
                copy_kv(g, pl.multiple_of(2 * i * RB, 8), RB)
                mix_in(i)
                copy_kv(g, pl.multiple_of((2 * i + 1) * RB, 8), RB)
                return c

            lax.fori_loop(lo, hi, body, 0)

        def issue_kv_block(j):
            g = j // GH
            jj = j % GH

            def mix_gate_up(i):
                e = g * STEPS + i - GU_FIRST

                @pl.when(jnp.logical_and(e >= 0, e < NGU))
                def _():
                    rows = pl.ds(pl.multiple_of(e * GR, GR), GR)
                    pltpu.make_async_copy(wg_hbm.at[rows, :], wg_v.at[rows, :],
                                          sem.at[S_WG]).start(priority=0)
                    pltpu.make_async_copy(wu_hbm.at[rows, :], wu_v.at[rows, :],
                                          sem.at[S_WU]).start(priority=1)

            lo = jj * PER_BLOCK
            kv_steps(g, lo, jnp.minimum(lo + PER_BLOCK, STEPS), mix_gate_up)
            if REM:
                @pl.when(jj == GH - 1)
                def _():
                    copy_kv(g, NB * RB, REM)

        def issue_trail(k):
            for a, r, n, s, p in trail[cuts[k]:cuts[k + 1]]:
                src, dst = (wo_hbm, wo_v) if a == "o" else (wd_hbm, wd_v)
                pltpu.make_async_copy(src.at[:, pl.ds(r, n), :], dst.at[:, pl.ds(r, n), :],
                                      sem.at[s]).start(priority=p)

        cp_x = pltpu.make_async_copy(x_hbm, x_v, sem.at[S_X])
        cp_wr = pltpu.make_async_copy(wr_hbm, wr_v, sem.at[S_WR])
        cp_x.start(priority=0)
        cp_wr.start(priority=1)

        def wq_small(j, c):
            per_tile = H * Dh // QC0
            copy_wq(slice(None), j // per_tile, pl.multiple_of((j % per_tile) * QC0, QC0), QC0)
            return c

        lax.fori_loop(0, QSM * (H * Dh // QC0), wq_small, 0)

        def mix_wq(i):
            @pl.when(i < 2 * QT * QQ)
            def _():
                k = i % (2 * QT)
                copy_wq(i // (2 * QT), QSM + k // 2, pl.multiple_of((k % 2) * QH, QH), QH)

        kv_steps(0, 0, STEPS, mix_wq)
        if REM:
            copy_kv(0, NB * RB, REM)

        cp_x.wait()
        x = x_v[0].astype(f32)
        mu = jnp.mean(x, axis=-1, keepdims=True)
        var = jnp.mean((x - mu) * (x - mu), axis=-1, keepdims=True)
        xn = _rnd(_rnd(x - _rnd(mu)) / _rnd(jnp.sqrt(_rnd(_rnd(var) + eps))))
        xn_s[...] = jnp.broadcast_to(xn, (M, D))
        cp_wr.wait()
        rr = jnp.zeros((1, Dh), f32)
        for j in range(D // Dh):
            rr = rr + xn[:, j * Dh:(j + 1) * Dh] * wr_v[j:j + 1, :].astype(f32)
        r_gate = _rnd(jax.nn.sigmoid(_rnd(jnp.sum(rr, axis=-1, keepdims=True))))

        for j in range(GH, LOOK):
            issue_kv_block(j)

        wait_all(wq_v, S_WQ)
        q = lax.dot_general(xn_s[...].astype(bf16), wq_v[...].reshape(D, H * Dh), _NN,
                            preferred_element_type=f32)
        for h in range(H):
            q_s[h] = q[:, h * Dh:(h + 1) * Dh]

        def head(h, carry):
            @pl.when(h < H - LOOK)
            def _():
                issue_kv_block(h + LOOK)

            for k in range(GH):
                @pl.when(h == H - GH + k)
                def _():
                    issue_trail(k)

            @pl.when(h == GU_HEAD)
            def _():
                xb = xn_s[...].astype(bf16)
                wait_all(wg_v, S_WG)
                gt = _rnd(lax.dot_general(xb, wg_v[...], _NT, preferred_element_type=f32))
                gt = _rnd(gt * jax.nn.sigmoid(gt))
                wait_all(wu_v, S_WU)
                up = lax.dot_general(xb, wu_v[...], _NT, preferred_element_type=f32)
                hid_s[...] = gt * _rnd(up)

            g = h // GH
            hh = h % GH

            @pl.when(hh == 0)
            def _():
                wait_all(kv_v.at[g], S_KV + g)

            qh = q_s[h].astype(bf16)
            s = lax.dot_general(qh, kv_v[g, 0, hh], _NT, preferred_element_type=f32)
            s = _rnd(_rnd(s) * scale)
            p = jnp.exp(s - jnp.max(s, axis=-1, keepdims=True))
            p = p * (1.0 / jnp.sum(p, axis=-1, keepdims=True))
            o_s[h] = lax.dot_general(p.astype(bf16), kv_v[g, 1, hh], _NN, preferred_element_type=f32)
            return carry

        lax.fori_loop(0, H, head, 0)

        issue_trail(GH)
        wait_all(wd_v, S_WD)
        y = lax.dot_general(hid_s[...].astype(bf16), wd_v[...].reshape(F, D), _NN,
                            preferred_element_type=f32)
        z = _rnd(xn + _rnd(_rnd(y) * r_gate))
        gate = _rnd(z * jax.nn.sigmoid(z))
        x_rep = jnp.broadcast_to(x, (M, D))

        o_all = jnp.concatenate([o_s[h] for h in range(H)], axis=1)
        lhs = [
            jnp.concatenate([o_all[:, i * OS + a0:i * OS + a1] for i in range(OQ)], axis=1).astype(bf16)
            for _, a0, a1 in chunks[:NMX]
        ]
        pick = (lax.broadcasted_iota(jnp.int32, (NV, Dh), 1)
                == lax.broadcasted_iota(jnp.int32, (NV, Dh), 0) + v0 % Dh)
        diag = jnp.concatenate([
            jnp.where(pick, jnp.broadcast_to(o_s[(i * OS + v0) // Dh][0:1], (NV, Dh)), 0.0)
            for i in range(OQ)], axis=0).astype(bf16)
        oc_s[...] = lax.dot_general(diag, jnp.ones((Dh, Dh), bf16), _NN, preferred_element_type=f32)

        for c, (_, a0, a1) in enumerate(chunks[:NMX]):
            wait_all(wo_v.at[:, pl.ds(a0, a1 - a0), :], S_WO + c)
            part = lax.dot_general(lhs[c], wo_v[:, a0:a1, :].reshape(OQ * (a1 - a0), D), _NN,
                                   preferred_element_type=f32)
            if c == 0:
                acc_s[...] = part
            elif c < NMX - 1:
                acc_s[...] += part
            else:
                res = x_rep + (acc_s[...] + part) * gate

        terms = []
        for c in range(NMX, NCH):
            _, a0, a1 = chunks[c]
            wait_all(wo_v.at[:, pl.ds(a0, a1 - a0), :], S_WO + c)
            for i in range(OQ):
                for r in range(a0, a1, 8):
                    oc = oc_s[pl.ds(i * NV + r - v0, 8), :]
                    terms.insert(0, wo_v[i, r:r + 8, :].astype(f32)
                                 * jnp.concatenate([oc] * (D // Dh), axis=1))
            while len(terms) > 1:
                terms = [terms[k] + terms[k + 1] if k + 1 < len(terms) else terms[k]
                         for k in range(0, len(terms), 2)]
        res = res[0:1] + jnp.sum(terms[0], axis=0, keepdims=True) * gate[0:1]
        o_ref[0] = res.astype(o_ref.dtype)

    params = dict(vmem_limit_bytes=100 * 1024 * 1024, disable_bounds_checks=True)
    try:
        compiler_params = pltpu.CompilerParams(disable_semaphore_checks=True, **params)
    except TypeError:
        compiler_params = pltpu.CompilerParams(**params)

    any_spec = pl.BlockSpec(memory_space=pl.ANY)
    return pl.pallas_call(
        kernel,
        out_shape=jax.ShapeDtypeStruct((B, Sq, D), A_x.dtype),
        in_specs=[any_spec] * 9,
        out_specs=pl.BlockSpec(memory_space=pltpu.VMEM),
        scratch_shapes=[
            pltpu.VMEM((1, 1, D), bf16),
            pltpu.VMEM((D // Dh, Dh), bf16),
            pltpu.VMEM((QQ, QS, H * Dh), bf16),
            pltpu.VMEM((OQ, OS, D), bf16),
            pltpu.VMEM((F, D), bf16),
            pltpu.VMEM((F, D), bf16),
            pltpu.VMEM((DQ, DS, D), bf16),
            pltpu.VMEM((G, 2, GH, W, Dh), bf16),
            pltpu.VMEM((H, M, Dh), f32),
            pltpu.VMEM((H, M, Dh), f32),
            pltpu.VMEM((M, D), f32),
            pltpu.VMEM((OQ * NV, Dh), f32),
            pltpu.VMEM((M, D), f32),
            pltpu.VMEM((M, F), f32),
            pltpu.SemaphoreType.DMA((NSEM,)),
        ],
        compiler_params=compiler_params,
    )(A_x, A_k_cache, A_v_cache,
      A_wq.reshape(QQ, QS, H * Dh), A_wo.reshape(OQ, OS, D), B_w_r.reshape(D // Dh, Dh),
      B_w_gate.T, B_w_up.T, B_w_down.reshape(DQ, DS, D))
```

```python
import jax
import jax.numpy as jnp
import numpy as np
from jax import lax
import jax.experimental.pallas as pl
import jax.experimental.pallas.tpu as pltpu

_NT = (((1,), (1,)), ((), ()))
_NN = (((1,), (0,)), ((), ()))

GH = 4
RB = 40
HP = 2
LOOK = 6
QQ = 4
QSM, QC0 = 4, 128
FR = 16
FFN_FIRST = 64
FFN_HEAD = 20
OQ, OR = 4, 8
WO_MXU = (((0, 384), (1, 128)), ((0, 128), (1, 128)), ((1, 128),), ((1, 64),))
WO_VPU = ((1, 32), (1, 24), (1, 8))
WO_ISSUE = (28, 80, 20)


def _rnd(a):
    return a.astype(jnp.bfloat16).astype(jnp.float32)


def _bf16_const(v):
    return float(np.asarray(v, dtype=jnp.bfloat16))


@jax.jit
def pallas_recurrent_scan__sliding_block_cached__moe_arch_mod__decode_kernel(
    A_x: jax.Array,
    A_k_cache: jax.Array,
    A_v_cache: jax.Array,
    A_wq: jax.Array,
    A_wo: jax.Array,
    B_x: jax.Array,
    B_w_r: jax.Array,
    B_w_gate: jax.Array,
    B_w_up: jax.Array,
    B_w_down: jax.Array,
):
    B, Sq, D = A_x.shape
    H, Dh = 32, 128
    Hkv, Sk = A_k_cache.shape[1], A_k_cache.shape[2]
    assert B == 1 and Sq == 1 and Hkv == H
    W = min(4096, max(256, Sk // 4))
    F = B_w_gate.shape[1]
    f32, bf16 = jnp.float32, jnp.bfloat16
    M = 8
    scale = _bf16_const(Dh ** -0.5)
    eps = _bf16_const(1e-5)
    G = H // GH
    OS, QS = H * Dh // OQ, D // QQ

    S_X, S_WR, S_WQ, S_WG, S_WU, S_WD, S_KV = 0, 1, 2, 3, 4, 5, 6
    S_WO = S_KV + G
    flat = [pc for step in WO_MXU for pc in step] + list(WO_VPU)
    assert sum(n for _, n in flat) == OS and all(n % OR == 0 for _, n in flat)
    nxt = [0, sum(n for t, n in flat if t == 0)]
    pieces = []
    streams = ([], [])
    for c, (t, n) in enumerate(flat):
        pieces.append((nxt[t], nxt[t] + n, S_WO + c))
        streams[t].extend((r, S_WO + c, t) for r in range(nxt[t], nxt[t] + n, OR))
        nxt[t] += n
    NSEM = S_WO + len(flat)
    mxu_steps, c = [], 0
    for step in WO_MXU:
        mxu_steps.append(pieces[c:c + len(step)])
        c += len(step)
    vpu_steps = pieces[c:]
    v0, v1 = vpu_steps[0][0], vpu_steps[-1][1]
    NV = v1 - v0
    assert NV == sum(n for _, n in WO_VPU) and v0 // Dh == (v1 - 1) // Dh and OS % Dh == 0
    wo_descs = []
    for i in range(max(len(s) for s in streams)):
        wo_descs.extend(s[i] for s in streams if i < len(s))
    cuts = [0]
    for n in WO_ISSUE:
        cuts.append(min(cuts[-1] + n, len(wo_descs)))
    cuts.append(len(wo_descs))

    NB = W // RB
    REM = W - NB * RB
    STEPS = NB // 2
    PER_BLOCK = -(-STEPS // GH)
    NF = F // FR
    QH = H * Dh // 2
    QT = QS // 16 - QSM
    assert NB % 2 == 0 and RB % 8 == 0 and REM % 8 == 0 and F % (2 * FR) == 0
    assert GH % HP == 0 and LOOK % HP == 0 and FFN_HEAD % HP == 0
    assert LOOK >= GH and HP * len(WO_ISSUE) <= LOOK and 2 * QT * QQ <= STEPS
    assert STEPS <= FFN_FIRST and FFN_FIRST + NF + NF // 2 <= (FFN_HEAD // GH) * STEPS
    assert FFN_HEAD + HP < H

    def kernel(x_hbm, k_hbm, v_hbm, wq_hbm, wo_hbm, wr_hbm, wg_hbm, wu_hbm, wd_hbm,
               o_ref,
               x_v, wr_v, wq_v, wo_v, wg_v, wu_v, wd_v, kv_v,
               q_s, o_s, acc_s, oc_s, xn_s, hid_s, gate_s, sem):

        def wait_all(buf, s):
            pltpu.make_async_copy(buf, buf, sem.at[s]).wait()

        def copy_kv(g, r, n):
            for p, src in ((0, k_hbm), (1, v_hbm)):
                pltpu.make_async_copy(
                    src.at[0, pl.ds(g * GH, GH), pl.ds(Sk - W + r, n), :],
                    kv_v.at[g, p, :, pl.ds(r, n), :],
                    sem.at[S_KV + g]).start(priority=p)

        def copy_wq(slabs, tile, col, n):
            for p in (0, 1):
                r = pl.multiple_of(p * (QS // 2) + tile * 8, 8)
                pltpu.make_async_copy(wq_hbm.at[slabs, pl.ds(r, 8), pl.ds(col, n)],
                                      wq_v.at[slabs, pl.ds(r, 8), pl.ds(col, n)],
                                      sem.at[S_WQ]).start(priority=p)

        def copy_ffn(src, dst, i, s, p):
            rows = pl.ds(pl.multiple_of(i * FR, FR), FR)
            pltpu.make_async_copy(src.at[rows, :], dst.at[rows, :], sem.at[s]).start(priority=p)

        def kv_steps(g, lo, hi, mix_in):
            def body(i, c):
                copy_kv(g, pl.multiple_of(2 * i * RB, 8), RB)
                mix_in(i)
                copy_kv(g, pl.multiple_of((2 * i + 1) * RB, 8), RB)
                return c

            lax.fori_loop(lo, hi, body, 0)

        def issue_kv_block(j):
            g = j // GH
            jj = j % GH

            def mix_ffn(i):
                e = g * STEPS + i - FFN_FIRST

                @pl.when(jnp.logical_and(e >= 0, e < NF))
                def _():
                    copy_ffn(wg_hbm, wg_v, e, S_WG, 0)
                    copy_ffn(wu_hbm, wu_v, e, S_WU, 1)

                @pl.when(jnp.logical_and(e >= NF, e < NF + NF // 2))
                def _():
                    copy_ffn(wd_hbm, wd_v, e - NF, S_WD, 0)
                    copy_ffn(wd_hbm, wd_v, e - NF // 2, S_WD, 1)

            lo = jj * PER_BLOCK
            kv_steps(g, lo, jnp.minimum(lo + PER_BLOCK, STEPS), mix_ffn)
            if REM:
                @pl.when(jj == GH - 1)
                def _():
                    copy_kv(g, NB * RB, REM)

        def issue_wo(k):
            for r, s, p in wo_descs[cuts[k]:cuts[k + 1]]:
                pltpu.make_async_copy(wo_hbm.at[:, pl.ds(r, OR), :], wo_v.at[:, pl.ds(r, OR), :],
                                      sem.at[s]).start(priority=p)

        def wait_wo(piece):
            a0, a1, s = piece
            wait_all(wo_v.at[:, pl.ds(a0, a1 - a0), :], s)

        cp_x = pltpu.make_async_copy(x_hbm, x_v, sem.at[S_X])
        cp_wr = pltpu.make_async_copy(wr_hbm, wr_v, sem.at[S_WR])
        cp_x.start(priority=0)
        cp_wr.start(priority=1)

        def wq_small(j, c):
            per_tile = H * Dh // QC0
            copy_wq(slice(None), j // per_tile, pl.multiple_of((j % per_tile) * QC0, QC0), QC0)
            return c

        lax.fori_loop(0, QSM * (H * Dh // QC0), wq_small, 0)

        def mix_wq(i):
            @pl.when(i < 2 * QT * QQ)
            def _():
                k = i % (2 * QT)
                copy_wq(i // (2 * QT), QSM + k // 2, pl.multiple_of((k % 2) * QH, QH), QH)

        kv_steps(0, 0, STEPS, mix_wq)
        if REM:
            copy_kv(0, NB * RB, REM)

        cp_x.wait()
        x = x_v[0].astype(f32)
        mu = jnp.mean(x, axis=-1, keepdims=True)
        var = jnp.mean((x - mu) * (x - mu), axis=-1, keepdims=True)
        xn = _rnd(_rnd(x - _rnd(mu)) / _rnd(jnp.sqrt(_rnd(_rnd(var) + eps))))
        xn_s[...] = jnp.broadcast_to(xn, (M, D))
        cp_wr.wait()
        rr = jnp.zeros((1, Dh), f32)
        for j in range(D // Dh):
            rr = rr + xn[:, j * Dh:(j + 1) * Dh] * wr_v[j:j + 1, :].astype(f32)
        r_sel = _rnd(jax.nn.sigmoid(_rnd(jnp.sum(rr, axis=-1, keepdims=True))))
        gate_s[...] = jnp.broadcast_to(r_sel, (M, D))

        for j in range(GH, LOOK):
            issue_kv_block(j)

        wait_all(wq_v, S_WQ)
        q = lax.dot_general(xn_s[...].astype(bf16), wq_v[...].reshape(D, H * Dh), _NN,
                            preferred_element_type=f32)
        for h in range(H):
            q_s[h] = q[:, h * Dh:(h + 1) * Dh]

        def scores(h):
            return lax.dot_general(q_s[h].astype(bf16), kv_v[h // GH, 0, h % GH], _NT,
                                   preferred_element_type=f32)

        def attend(h, s):
            s = _rnd(_rnd(s) * scale)
            p = jnp.exp(s - jnp.max(s, axis=-1, keepdims=True))
            p = p * (1.0 / jnp.sum(p, axis=-1, keepdims=True))
            return lax.dot_general(p.astype(bf16), kv_v[h // GH, 1, h % GH], _NN,
                                   preferred_element_type=f32)

        def heads(t, carry):
            h = t * HP

            @pl.when(h < H - LOOK)
            def _():
                def block(u, c):
                    issue_kv_block(h + LOOK + u)
                    return c

                lax.fori_loop(0, HP, block, 0)

            for k in range(len(WO_ISSUE)):
                @pl.when(h == H - HP * (len(WO_ISSUE) - k))
                def _():
                    issue_wo(k)

            @pl.when(h == FFN_HEAD)
            def _():
                xb = xn_s[...].astype(bf16)
                wait_all(wg_v, S_WG)
                gt = _rnd(lax.dot_general(xb, wg_v[...], _NT, preferred_element_type=f32))
                gt = _rnd(gt * jax.nn.sigmoid(gt))
                wait_all(wu_v, S_WU)
                up = lax.dot_general(xb, wu_v[...], _NT, preferred_element_type=f32)
                hid_s[...] = gt * _rnd(up)

            @pl.when(h == FFN_HEAD + HP)
            def _():
                wait_all(wd_v, S_WD)
                y = lax.dot_general(hid_s[...].astype(bf16), wd_v[...], _NN,
                                    preferred_element_type=f32)
                z = _rnd(xn_s[...] + _rnd(_rnd(y) * gate_s[...]))
                gate_s[...] = _rnd(z * jax.nn.sigmoid(z))

            @pl.when(h % GH == 0)
            def _():
                wait_all(kv_v.at[h // GH], S_KV + h // GH)

            ss = [scores(h + u) for u in range(HP)]
            outs = [attend(h + u, ss[u]) for u in range(HP)]
            for u in range(HP):
                o_s[h + u] = outs[u]
            return carry

        lax.fori_loop(0, H // HP, heads, 0)
        issue_wo(len(WO_ISSUE))

        gate = gate_s[...]
        for k, step in enumerate(mxu_steps):
            for piece in step:
                wait_wo(piece)
            if k == 0:
                o_all = jnp.concatenate([o_s[h] for h in range(H)], axis=1)
                pick = (lax.broadcasted_iota(jnp.int32, (NV, Dh), 1)
                        == lax.broadcasted_iota(jnp.int32, (NV, Dh), 0) + v0 % Dh)
                diag = jnp.concatenate([
                    jnp.where(pick, jnp.broadcast_to(o_s[(i * OS + v0) // Dh][0:1], (NV, Dh)), 0.0)
                    for i in range(OQ)], axis=0).astype(bf16)
                oc_s[...] = lax.dot_general(diag, jnp.ones((Dh, Dh), bf16), _NN,
                                            preferred_element_type=f32)
                lhs = [jnp.concatenate([o_all[:, i * OS + a0:i * OS + a1]
                                        for a0, a1, _ in st for i in range(OQ)], axis=1).astype(bf16)
                       for st in mxu_steps]
            rhs = jnp.concatenate([wo_v[:, a0:a1, :].reshape(OQ * (a1 - a0), D)
                                   for a0, a1, _ in step], axis=0)
            part = lax.dot_general(lhs[k], rhs, _NN, preferred_element_type=f32)
            if k == 0:
                acc_s[...] = part
            elif k < len(mxu_steps) - 1:
                acc_s[...] += part
            else:
                res = jnp.broadcast_to(x, (M, D)) + (acc_s[...] + part) * gate

        terms = []
        for piece in vpu_steps:
            wait_wo(piece)
            for i in range(OQ):
                for r in range(piece[0], piece[1], 8):
                    oc = oc_s[pl.ds(i * NV + r - v0, 8), :]
                    terms.insert(0, wo_v[i, r:r + 8, :].astype(f32)
                                 * jnp.concatenate([oc] * (D // Dh), axis=1))
            while len(terms) > 1:
                terms = [terms[k] + terms[k + 1] if k + 1 < len(terms) else terms[k]
                         for k in range(0, len(terms), 2)]
        res = res[0:1] + jnp.sum(terms[0], axis=0, keepdims=True) * gate[0:1]
        o_ref[0] = res.astype(o_ref.dtype)

    params = dict(vmem_limit_bytes=100 * 1024 * 1024, disable_bounds_checks=True)
    try:
        compiler_params = pltpu.CompilerParams(disable_semaphore_checks=True, **params)
    except TypeError:
        compiler_params = pltpu.CompilerParams(**params)

    any_spec = pl.BlockSpec(memory_space=pl.ANY)
    return pl.pallas_call(
        kernel,
        out_shape=jax.ShapeDtypeStruct((B, Sq, D), A_x.dtype),
        in_specs=[any_spec] * 9,
        out_specs=pl.BlockSpec(memory_space=pltpu.VMEM),
        scratch_shapes=[
            pltpu.VMEM((1, 1, D), bf16),
            pltpu.VMEM((D // Dh, Dh), bf16),
            pltpu.VMEM((QQ, QS, H * Dh), bf16),
            pltpu.VMEM((OQ, OS, D), bf16),
            pltpu.VMEM((F, D), bf16),
            pltpu.VMEM((F, D), bf16),
            pltpu.VMEM((F, D), bf16),
            pltpu.VMEM((G, 2, GH, W, Dh), bf16),
            pltpu.VMEM((H, M, Dh), f32),
            pltpu.VMEM((H, M, Dh), f32),
            pltpu.VMEM((M, D), f32),
            pltpu.VMEM((OQ * NV, Dh), f32),
            pltpu.VMEM((M, D), f32),
            pltpu.VMEM((M, F), f32),
            pltpu.VMEM((M, D), f32),
            pltpu.SemaphoreType.DMA((NSEM,)),
        ],
        compiler_params=compiler_params,
    )(A_x, A_k_cache, A_v_cache,
      A_wq.reshape(QQ, QS, H * Dh), A_wo.reshape(OQ, OS, D), B_w_r.reshape(D // Dh, Dh),
      B_w_gate.T, B_w_up.T, B_w_down)
```

```python
import jax
import jax.numpy as jnp
import numpy as np
from jax import lax
import jax.experimental.pallas as pl
import jax.experimental.pallas.tpu as pltpu

_NT = (((1,), (1,)), ((), ()))
_NN = (((1,), (0,)), ((), ()))

KV_KINDS = ((6, 16, 4), (4, 40, 2))
HP = 2
LOOK = 8
QQ = 4
QSM, QC0 = 4, 128
FR = 16
FFN_FIRST = 140
FFN_HEAD = 18
OQ, OR = 4, 8
WO_MXU = (((0, 384), (1, 128)), ((0, 128), (1, 128)), ((1, 128),), ((1, 64),))
WO_VPU = ((1, 32), (1, 24), (1, 8))
WO_ISSUE = (28, 28, 52, 20)


def _rnd(a):
    return a.astype(jnp.bfloat16).astype(jnp.float32)


def _bf16_const(v):
    return float(np.asarray(v, dtype=jnp.bfloat16))


@jax.jit
def pallas_recurrent_scan__sliding_block_cached__moe_arch_mod__decode_kernel(
    A_x: jax.Array,
    A_k_cache: jax.Array,
    A_v_cache: jax.Array,
    A_wq: jax.Array,
    A_wo: jax.Array,
    B_x: jax.Array,
    B_w_r: jax.Array,
    B_w_gate: jax.Array,
    B_w_up: jax.Array,
    B_w_down: jax.Array,
):
    B, Sq, D = A_x.shape
    H, Dh = 32, 128
    Hkv, Sk = A_k_cache.shape[1], A_k_cache.shape[2]
    assert B == 1 and Sq == 1 and Hkv == H
    W = min(4096, max(256, Sk // 4))
    F = B_w_gate.shape[1]
    f32, bf16 = jnp.float32, jnp.bfloat16
    M = 8
    scale = _bf16_const(Dh ** -0.5)
    eps = _bf16_const(1e-5)
    G = sum(n for _, _, n in KV_KINDS)
    OS, QS = H * Dh // OQ, D // QQ

    S_X, S_WR, S_WQ, S_WG, S_WU, S_WD, S_KV = 0, 1, 2, 3, 4, 5, 6
    S_WO = S_KV + G
    flat = [pc for step in WO_MXU for pc in step] + list(WO_VPU)
    assert sum(n for _, n in flat) == OS and all(n % OR == 0 for _, n in flat)
    nxt = [0, sum(n for t, n in flat if t == 0)]
    pieces = []
    streams = ([], [])
    for c, (t, n) in enumerate(flat):
        pieces.append((nxt[t], nxt[t] + n, S_WO + c))
        streams[t].extend((r, S_WO + c, t) for r in range(nxt[t], nxt[t] + n, OR))
        nxt[t] += n
    NSEM = S_WO + len(flat)
    mxu_steps, c = [], 0
    for step in WO_MXU:
        mxu_steps.append(pieces[c:c + len(step)])
        c += len(step)
    vpu_steps = pieces[c:]
    v0, v1 = vpu_steps[0][0], vpu_steps[-1][1]
    NV = v1 - v0
    assert NV == sum(n for _, n in WO_VPU) and v0 // Dh == (v1 - 1) // Dh and OS % Dh == 0
    wo_descs = []
    for i in range(max(len(s) for s in streams)):
        wo_descs.extend(s[i] for s in streams if i < len(s))
    cuts = [0]
    for n in WO_ISSUE:
        cuts.append(min(cuts[-1] + n, len(wo_descs)))
    cuts.append(len(wo_descs))

    kinds = []
    h0 = g0 = 0
    for nh, rb, n in KV_KINDS:
        assert rb % 8 == 0 and nh % HP == 0 and LOOK >= nh
        kinds.append((nh, rb, h0, h0 + n * nh, g0, W // (2 * rb)))
        h0, g0 = h0 + n * nh, g0 + n
    assert h0 == H and W % 8 == 0
    GH, STEPS = kinds[0][0], kinds[0][5]
    NF = F // FR
    QH = H * Dh // 2
    QT = QS // 16 - QSM
    assert F % (2 * FR) == 0 and LOOK % HP == 0 and FFN_HEAD % HP == 0
    assert HP * len(WO_ISSUE) <= LOOK <= kinds[0][3] and 4 * QT * QQ <= STEPS
    assert STEPS <= FFN_FIRST and FFN_FIRST + NF + NF // 2 <= (FFN_HEAD // GH) * STEPS
    assert FFN_HEAD <= kinds[0][3] and FFN_HEAD + HP < H

    def kernel(x_hbm, k_hbm, v_hbm, wq_hbm, wo_hbm, wr_hbm, wg_hbm, wu_hbm, wd_hbm,
               o_ref,
               x_v, wr_v, wq_v, wo_v, wg_v, wu_v, wd_v, kv_v,
               q_s, o_s, acc_s, oc_s, xn_s, hid_s, gate_s, sem):

        def wait_all(buf, s):
            pltpu.make_async_copy(buf, buf, sem.at[s]).wait()

        def copy_kv(kind, gi, r, n):
            nh, _, first_head, _, first_group, _ = kind
            heads_ = pl.ds(first_head + gi * nh, nh)
            for p, src in ((0, k_hbm), (1, v_hbm)):
                pltpu.make_async_copy(
                    src.at[0, heads_, pl.ds(Sk - W + r, n), :],
                    kv_v.at[p, heads_, pl.ds(r, n), :],
                    sem.at[S_KV + first_group + gi]).start(priority=p)

        def copy_wq(slabs, tile, col, n):
            for p in (0, 1):
                r = pl.multiple_of(p * (QS // 2) + tile * 8, 8)
                pltpu.make_async_copy(wq_hbm.at[slabs, pl.ds(r, 8), pl.ds(col, n)],
                                      wq_v.at[slabs, pl.ds(r, 8), pl.ds(col, n)],
                                      sem.at[S_WQ]).start(priority=p)

        def copy_ffn(src, dst, i, s, p):
            rows = pl.ds(pl.multiple_of(i * FR, FR), FR)
            pltpu.make_async_copy(src.at[rows, :], dst.at[rows, :], sem.at[s]).start(priority=p)

        def kv_steps(kind, gi, lo, hi, mix_in):
            rb = kind[1]

            def body(i, c):
                copy_kv(kind, gi, pl.multiple_of(2 * i * rb, 8), rb)
                mix_in(i)
                copy_kv(kind, gi, pl.multiple_of((2 * i + 1) * rb, 8), rb)
                return c

            lax.fori_loop(lo, hi, body, 0)

        def kv_leftover(kind, gi):
            rb, steps = kind[1], kind[5]
            for r in range(2 * steps * rb, W, rb):
                copy_kv(kind, gi, r, min(rb, W - r))

        def issue_kv_block(kind, j):
            nh, _, first_head, _, _, steps = kind
            gi = (j - first_head) // nh
            jj = (j - first_head) % nh

            def mix_ffn(i):
                if kind is not kinds[0]:
                    return
                e = gi * STEPS + i - FFN_FIRST

                @pl.when(jnp.logical_and(e >= 0, e < NF))
                def _():
                    copy_ffn(wg_hbm, wg_v, e, S_WG, 0)
                    copy_ffn(wu_hbm, wu_v, e, S_WU, 1)

                @pl.when(jnp.logical_and(e >= NF, e < NF + NF // 2))
                def _():
                    copy_ffn(wd_hbm, wd_v, e - NF, S_WD, 0)
                    copy_ffn(wd_hbm, wd_v, e - NF // 2, S_WD, 1)

            per_block = -(-steps // nh)
            lo = jj * per_block
            kv_steps(kind, gi, lo, jnp.minimum(lo + per_block, steps), mix_ffn)

            @pl.when(jj == nh - 1)
            def _():
                kv_leftover(kind, gi)

        def issue_wo(k):
            for r, s, p in wo_descs[cuts[k]:cuts[k + 1]]:
                pltpu.make_async_copy(wo_hbm.at[:, pl.ds(r, OR), :], wo_v.at[:, pl.ds(r, OR), :],
                                      sem.at[s]).start(priority=p)

        def wait_wo(piece):
            a0, a1, s = piece
            wait_all(wo_v.at[:, pl.ds(a0, a1 - a0), :], s)

        cp_x = pltpu.make_async_copy(x_hbm, x_v, sem.at[S_X])
        cp_wr = pltpu.make_async_copy(wr_hbm, wr_v, sem.at[S_WR])
        cp_x.start(priority=0)
        cp_wr.start(priority=1)

        def wq_small(j, c):
            per_tile = H * Dh // QC0
            copy_wq(slice(None), j // per_tile, pl.multiple_of((j % per_tile) * QC0, QC0), QC0)
            return c

        lax.fori_loop(0, QSM * (H * Dh // QC0), wq_small, 0)

        def mix_wq(i):
            @pl.when(jnp.logical_and(i % 2 == 0, i < 4 * QT * QQ))
            def _():
                k = (i // 2) % (2 * QT)
                copy_wq(i // (4 * QT), QSM + k // 2, pl.multiple_of((k % 2) * QH, QH), QH)

        kv_steps(kinds[0], 0, 0, STEPS, mix_wq)
        kv_leftover(kinds[0], 0)

        cp_x.wait()
        x = x_v[0].astype(f32)
        mu = jnp.mean(x, axis=-1, keepdims=True)
        var = jnp.mean((x - mu) * (x - mu), axis=-1, keepdims=True)
        xn = _rnd(_rnd(x - _rnd(mu)) / _rnd(jnp.sqrt(_rnd(_rnd(var) + eps))))
        xn_s[...] = jnp.broadcast_to(xn, (M, D))
        cp_wr.wait()
        rr = jnp.zeros((1, Dh), f32)
        for j in range(D // Dh):
            rr = rr + xn[:, j * Dh:(j + 1) * Dh] * wr_v[j:j + 1, :].astype(f32)
        r_sel = _rnd(jax.nn.sigmoid(_rnd(jnp.sum(rr, axis=-1, keepdims=True))))
        gate_s[...] = jnp.broadcast_to(r_sel, (M, D))

        for j in range(GH, LOOK):
            issue_kv_block(kinds[0], j)

        wait_all(wq_v, S_WQ)
        q = lax.dot_general(xn_s[...].astype(bf16), wq_v[...].reshape(D, H * Dh), _NN,
                            preferred_element_type=f32)
        for h in range(H):
            q_s[h] = q[:, h * Dh:(h + 1) * Dh]

        def scores(h):
            return lax.dot_general(q_s[h].astype(bf16), kv_v[0, h], _NT,
                                   preferred_element_type=f32)

        def attend(h, s):
            s = _rnd(_rnd(s) * scale)
            p = jnp.exp(s - jnp.max(s, axis=-1, keepdims=True))
            p = p * (1.0 / jnp.sum(p, axis=-1, keepdims=True))
            return lax.dot_general(p.astype(bf16), kv_v[1, h], _NN,
                                   preferred_element_type=f32)

        def heads(t, carry):
            h = t * HP

            for kind in kinds:
                @pl.when(jnp.logical_and(h + LOOK >= kind[2], h + LOOK < kind[3]))
                def _():
                    def block(u, c):
                        issue_kv_block(kind, h + LOOK + u)
                        return c

                    lax.fori_loop(0, HP, block, 0)

            for k in range(len(WO_ISSUE)):
                @pl.when(h == H - HP * (len(WO_ISSUE) - k))
                def _():
                    issue_wo(k)

            @pl.when(h == FFN_HEAD)
            def _():
                xb = xn_s[...].astype(bf16)
                wait_all(wg_v, S_WG)
                gt = _rnd(lax.dot_general(xb, wg_v[...], _NT, preferred_element_type=f32))
                gt = _rnd(gt * jax.nn.sigmoid(gt))
                wait_all(wu_v, S_WU)
                up = lax.dot_general(xb, wu_v[...], _NT, preferred_element_type=f32)
                hid_s[...] = gt * _rnd(up)

            @pl.when(h == FFN_HEAD + HP)
            def _():
                wait_all(wd_v, S_WD)
                y = lax.dot_general(hid_s[...].astype(bf16), wd_v[...], _NN,
                                    preferred_element_type=f32)
                z = _rnd(xn_s[...] + _rnd(_rnd(y) * gate_s[...]))
                gate_s[...] = _rnd(z * jax.nn.sigmoid(z))

            for nh, _, first_head, end_head, first_group, _ in kinds:
                @pl.when(jnp.logical_and(jnp.logical_and(h >= first_head, h < end_head),
                                         (h - first_head) % nh == 0))
                def _():
                    wait_all(kv_v.at[:, pl.ds(h, nh)], S_KV + first_group + (h - first_head) // nh)

            ss = [scores(h + u) for u in range(HP)]
            outs = [attend(h + u, ss[u]) for u in range(HP)]
            for u in range(HP):
                o_s[h + u] = outs[u]
            return carry

        lax.fori_loop(0, H // HP, heads, 0)
        issue_wo(len(WO_ISSUE))

        gate = gate_s[...]
        for k, step in enumerate(mxu_steps):
            for piece in step:
                wait_wo(piece)
            if k == 0:
                o_all = jnp.concatenate([o_s[h] for h in range(H)], axis=1)
                pick = (lax.broadcasted_iota(jnp.int32, (NV, Dh), 1)
                        == lax.broadcasted_iota(jnp.int32, (NV, Dh), 0) + v0 % Dh)
                diag = jnp.concatenate([
                    jnp.where(pick, jnp.broadcast_to(o_s[(i * OS + v0) // Dh][0:1], (NV, Dh)), 0.0)
                    for i in range(OQ)], axis=0).astype(bf16)
                oc_s[...] = lax.dot_general(diag, jnp.ones((Dh, Dh), bf16), _NN,
                                            preferred_element_type=f32)
                lhs = [jnp.concatenate([o_all[:, i * OS + a0:i * OS + a1]
                                        for a0, a1, _ in st for i in range(OQ)], axis=1).astype(bf16)
                       for st in mxu_steps]
            rhs = jnp.concatenate([wo_v[:, a0:a1, :].reshape(OQ * (a1 - a0), D)
                                   for a0, a1, _ in step], axis=0)
            part = lax.dot_general(lhs[k], rhs, _NN, preferred_element_type=f32)
            if k == 0:
                acc_s[...] = part
            elif k < len(mxu_steps) - 1:
                acc_s[...] += part
            else:
                res = jnp.broadcast_to(x, (M, D)) + (acc_s[...] + part) * gate

        terms = []
        for piece in vpu_steps:
            wait_wo(piece)
            for i in range(OQ):
                for r in range(piece[0], piece[1], 8):
                    oc = oc_s[pl.ds(i * NV + r - v0, 8), :]
                    terms.insert(0, wo_v[i, r:r + 8, :].astype(f32)
                                 * jnp.concatenate([oc] * (D // Dh), axis=1))
            while len(terms) > 1:
                terms = [terms[k] + terms[k + 1] if k + 1 < len(terms) else terms[k]
                         for k in range(0, len(terms), 2)]
        res = res[0:1] + jnp.sum(terms[0], axis=0, keepdims=True) * gate[0:1]
        o_ref[0] = res.astype(o_ref.dtype)

    params = dict(vmem_limit_bytes=100 * 1024 * 1024, disable_bounds_checks=True)
    try:
        compiler_params = pltpu.CompilerParams(disable_semaphore_checks=True, **params)
    except TypeError:
        compiler_params = pltpu.CompilerParams(**params)

    any_spec = pl.BlockSpec(memory_space=pl.ANY)
    return pl.pallas_call(
        kernel,
        out_shape=jax.ShapeDtypeStruct((B, Sq, D), A_x.dtype),
        in_specs=[any_spec] * 9,
        out_specs=pl.BlockSpec(memory_space=pltpu.VMEM),
        scratch_shapes=[
            pltpu.VMEM((1, 1, D), bf16),
            pltpu.VMEM((D // Dh, Dh), bf16),
            pltpu.VMEM((QQ, QS, H * Dh), bf16),
            pltpu.VMEM((OQ, OS, D), bf16),
            pltpu.VMEM((F, D), bf16),
            pltpu.VMEM((F, D), bf16),
            pltpu.VMEM((F, D), bf16),
            pltpu.VMEM((2, H, W, Dh), bf16),
            pltpu.VMEM((H, M, Dh), f32),
            pltpu.VMEM((H, M, Dh), f32),
            pltpu.VMEM((M, D), f32),
            pltpu.VMEM((OQ * NV, Dh), f32),
            pltpu.VMEM((M, D), f32),
            pltpu.VMEM((M, F), f32),
            pltpu.VMEM((M, D), f32),
            pltpu.SemaphoreType.DMA((NSEM,)),
        ],
        compiler_params=compiler_params,
    )(A_x, A_k_cache, A_v_cache,
      A_wq.reshape(QQ, QS, H * Dh), A_wo.reshape(OQ, OS, D), B_w_r.reshape(D // Dh, Dh),
      B_w_gate.T, B_w_up.T, B_w_down)
```
